```python
import os as _os
_os.environ.setdefault("JAX_PLATFORMS", "cpu")
import jax
import jax.numpy as jnp

def _softmax(x, axis=-1):
    return jax.nn.softmax(x, axis=axis)
def _gelu(x):
    return jax.nn.gelu(x, approximate=True)
def _silu(x):
    return jax.nn.silu(x)
def _sigmoid(x):
    return jax.nn.sigmoid(x)
def _layernorm(x, axis=-1, eps=1e-5):
    m = jnp.mean(x, axis=axis, keepdims=True)
    v = jnp.var(x, axis=axis, keepdims=True)
    return (x - m) / jnp.sqrt(v + eps)
def _scatter_add(tgt, idx, src, axis=0):
    return tgt.at[idx].add(src)
def _segment_sum(src, seg, n):
    return jax.ops.segment_sum(src, seg, n)
class _Rng:
    def __init__(self, key):
        self._k = key
    def _next(self):
        self._k, sub = jax.random.split(self._k)
        return sub
    def normal(self, shape):
        return jax.random.normal(self._next(), shape, dtype=jnp.bfloat16)
    def randint(self, lo, hi, shape):
        return jax.random.randint(self._next(), shape, lo, hi, dtype=jnp.int32)
    def uniform(self, shape, lo=0.0, hi=1.0):
        return jax.random.uniform(self._next(), shape, jnp.bfloat16, lo, hi)
    def permutation(self, n):
        return jax.random.permutation(self._next(), n)


kernel_name = 'sequential_preLN__softmax_full_mha__geglu_ffn__prompt'

def setup_inputs():
    _rng = _Rng(jax.random.key(int.from_bytes(__import__("os").urandom(4), "little")))
    _w = (lambda a: (lambda t: t.astype(jnp.bfloat16) if jnp.issubdtype(t.dtype, jnp.floating) else t)(jnp.asarray(a)))
    def _A_setup():
        B, S, D = 1, 2048, 512
        return {
            "x": _w((lambda *s: _rng.normal(s) * 0.05)(B, S, D)),
            "wqkv": _w((lambda *s: _rng.normal(s) * 0.05)(D, 3 * D)),
            "wo": _w((lambda *s: _rng.normal(s) * 0.05)(D, D)),
        }
    _A_in = _A_setup()

    def _B_setup():
        B, S, D, F = 1, 2048, 512, 1376
        return {
            "x": _w((lambda *s: _rng.normal(s) * 0.05)(B, S, D)),
            "w_gate": _w((lambda *s: _rng.normal(s) * 0.05)(D, F)),
            "w_up": _w((lambda *s: _rng.normal(s) * 0.05)(D, F)),
            "w_down": _w((lambda *s: _rng.normal(s) * 0.05)(F, D)),
        }
    _B_in = _B_setup()

    return {
        "A_x": _A_in["x"],
        "A_wqkv": _A_in["wqkv"],
        "A_wo": _A_in["wo"],
        "B_x": _B_in["x"],
        "B_w_gate": _B_in["w_gate"],
        "B_w_up": _B_in["w_up"],
        "B_w_down": _B_in["w_down"],
    }

def reference(A_x, A_wqkv, A_wo, B_x, B_w_gate, B_w_up, B_w_down):
    def _A_ref(x, wqkv, wo):
        B, S, D = x.shape
        H = 32; Dh = D // H
        qkv = (lambda x, *d: x.transpose(*d))((x @ wqkv).reshape(B, S, 3, H, Dh), 2, 0, 3, 1, 4)
        q, k, v = qkv[0], qkv[1], qkv[2]
        scale = Dh ** -0.5
        scores = jnp.einsum("bhqd,bhkd->bhqk", q, k) * scale
        p = _softmax(scores, axis=-1)
        o = jnp.einsum("bhqk,bhkd->bhqd", p, v)
        return (lambda x, *d: x.transpose(*d))(o, 0, 2, 1, 3).reshape(B, S, D) @ wo

    def _B_ref(x, w_gate, w_up, w_down):
        return (_gelu(x @ w_gate) * (x @ w_up)) @ w_down

    x = A_x
    h = x + _A_ref(_layernorm(x, axis=-1), A_wqkv, A_wo)
    h2 = h + _B_ref(_layernorm(h, axis=-1), B_w_gate, B_w_up, B_w_down)
    return h2
```

```python
import math

import jax
import jax.numpy as jnp
from jax import lax
import jax.experimental.pallas as pl
import jax.experimental.pallas.tpu as pltpu

S, D, H, DH, F = 2048, 512, 32, 16, 1376
TQ = 512
NQ = S // TQ
CK = 128
NC = S // CK
U = 4
HG = 128 // DH
EPS = 1e-5
QSCALE = (DH ** -0.5) * math.log2(math.e)
f32, bf16 = jnp.float32, jnp.bfloat16

NT = (((1,), (1,)), ((), ()))
TN = (((0,), (0,)), ((), ()))


def _layernorm(x):
    m = jnp.mean(x, axis=-1, keepdims=True)
    xc = x - m
    v = jnp.mean(xc * xc, axis=-1, keepdims=True)
    return xc * lax.rsqrt(v + EPS)


def _gelu_tanh(x):
    c = math.sqrt(2.0 / math.pi)
    return 0.5 * x * (1.0 + jnp.tanh(c * (x + 0.044715 * (x * x * x))))


def _kernel(x_hbm, wqkv_hbm, wo_hbm, wg_hbm, wu_hbm, wd_hbm, out_hbm,
            x_s, wqkv_s, wo_s, wg_s, wu_s, wd_s, wqvt_s, k_s, qt_s, vt_s,
            sbuf, mbuf, ot_s, out_s, sem_x, sem_w, sem_o):
    def x_copy(i):
        return pltpu.make_async_copy(
            x_hbm.at[pl.ds(i * TQ, TQ), :], x_s.at[pl.ds(i * TQ, TQ), :], sem_x.at[i])

    def out_copy(i):
        return pltpu.make_async_copy(
            out_s.at[pl.ds(i * TQ, TQ), :], out_hbm.at[pl.ds(i * TQ, TQ), :], sem_o.at[i])

    w_copies = [
        pltpu.make_async_copy(src, dst, sem_w.at[j])
        for j, (src, dst) in enumerate(
            [(wqkv_hbm, wqkv_s), (wo_hbm, wo_s), (wg_hbm, wg_s), (wu_hbm, wu_s), (wd_hbm, wd_s)])
    ]
    w_copies[0].start()
    for i in range(NQ):
        x_copy(i).start()
    for cp in w_copies[1:]:
        cp.start()

    w_copies[0].wait()
    wqvt_s[0:D, :] = wqkv_s[:, 0:D].T
    wqvt_s[D:2 * D, :] = wqkv_s[:, 2 * D:3 * D].T
    for i in range(NQ):
        x_copy(i).wait()
        xn = _layernorm(x_s[pl.ds(i * TQ, TQ), :].astype(f32)).astype(bf16)
        kk = jnp.dot(xn, wqkv_s[:, D:2 * D], preferred_element_type=f32).astype(bf16)
        for g in range(D // 128):
            k_s[g, pl.ds(i * TQ, TQ), :] = kk[:, g * 128:(g + 1) * 128]
        qv = lax.dot_general(wqvt_s[...], xn, NT, preferred_element_type=f32)
        qt_s[i] = (qv[0:D] * QSCALE).astype(bf16)
        vt_s[:, pl.ds(i * TQ, TQ)] = qv[D:2 * D].astype(bf16)

    T = NQ * H

    def stage(u, t_next, t_cur):
        if t_next is not None:
            hn = t_next % H
            g = hn // HG
            blk = qt_s[t_next // H, pl.ds(pl.multiple_of(g * 128, 128), 128), :]
            row = lax.broadcasted_iota(jnp.int32, (128, TQ), 0)
            w = jnp.where((row // DH) == (hn % HG), blk, jnp.zeros_like(blk))
        if t_cur is not None:
            hrow = pl.multiple_of((t_cur % H) * DH, DH)
            m_cur = mbuf[u]
            acc = jnp.zeros((DH, TQ), f32)
        mpart = None
        lpart = None
        for c in range(NC):
            if t_next is not None:
                s = jnp.dot(k_s[g, pl.ds(c * CK, CK), :], w, preferred_element_type=f32)
            if t_cur is not None:
                sc = sbuf[u, pl.ds(c * CK, CK), :].reshape(CK // 8, 8, TQ)
                p = jnp.exp2(sc - m_cur[None]).reshape(CK, TQ)
                loc = None
                for r in reversed(range(CK // 16)):
                    pair = p[r * 16:r * 16 + 8, :] + p[r * 16 + 8:r * 16 + 16, :]
                    loc = pair if loc is None else loc + pair
                lpart = loc if lpart is None else lpart + loc
                acc = acc + jnp.dot(vt_s[pl.ds(hrow, DH), pl.ds(c * CK, CK)],
                                    p.astype(bf16), preferred_element_type=f32)
            if t_next is not None:
                sbuf[u, pl.ds(c * CK, CK), :] = s
                for r in range(CK // 8):
                    srow = s[r * 8:(r + 1) * 8, :]
                    mpart = srow if mpart is None else jnp.maximum(mpart, srow)
        if t_cur is not None:
            l = jnp.sum(lpart, axis=0, keepdims=True)
            ot_s[t_cur // H, pl.ds(hrow, DH), :] = (acc * (1.0 / l)).astype(bf16)
        if t_next is not None:
            mbuf[u] = jnp.broadcast_to(jnp.max(mpart, axis=0, keepdims=True), (8, TQ))

    for u in range(U):
        stage(u, u, None)

    def body(i, carry):
        t = U * i
        for u in range(U):
            stage(u, t + U + u, t + u)
        return carry

    lax.fori_loop(0, T // U - 1, body, 0)
    for u in range(U):
        stage(u, None, T - U + u)

    for cp in w_copies[1:]:
        cp.wait()

    def ffn(i, carry):
        rows = pl.ds(pl.multiple_of(i * TQ, TQ), TQ)
        attn = lax.dot_general(ot_s[i], wo_s[...], TN, preferred_element_type=f32)
        h = x_s[rows, :].astype(f32) + attn
        hn = _layernorm(h).astype(bf16)
        gate = jnp.dot(hn, wg_s[...], preferred_element_type=f32)
        up = jnp.dot(hn, wu_s[...], preferred_element_type=f32)
        act = (_gelu_tanh(gate) * up).astype(bf16)
        y = h + jnp.dot(act, wd_s[...], preferred_element_type=f32)
        out_s[rows, :] = y.astype(bf16)
        out_copy(i).start()
        return carry

    lax.fori_loop(0, NQ, ffn, 0)
    for i in range(NQ):
        out_copy(i).wait()


@jax.jit
def pallas_sequential_preLN__softmax_full_mha__geglu_ffn__prompt_kernel(
    A_x: jax.Array,
    A_wqkv: jax.Array,
    A_wo: jax.Array,
    B_x: jax.Array,
    B_w_gate: jax.Array,
    B_w_up: jax.Array,
    B_w_down: jax.Array,
):
    del B_x
    any_spec = pl.BlockSpec(memory_space=pl.ANY)
    out = pl.pallas_call(
        _kernel,
        out_shape=jax.ShapeDtypeStruct((S, D), bf16),
        in_specs=[any_spec] * 6,
        out_specs=any_spec,
        scratch_shapes=[
            pltpu.VMEM((S, D), bf16),
            pltpu.VMEM((D, 3 * D), bf16),
            pltpu.VMEM((D, D), bf16),
            pltpu.VMEM((D, F), bf16),
            pltpu.VMEM((D, F), bf16),
            pltpu.VMEM((F, D), bf16),
            pltpu.VMEM((2 * D, D), bf16),
            pltpu.VMEM((D // 128, S, 128), bf16),
            pltpu.VMEM((NQ, D, TQ), bf16),
            pltpu.VMEM((D, S), bf16),
            pltpu.VMEM((U, S, TQ), f32),
            pltpu.VMEM((U, 8, TQ), f32),
            pltpu.VMEM((NQ, D, TQ), bf16),
            pltpu.VMEM((S, D), bf16),
            pltpu.SemaphoreType.DMA((NQ,)),
            pltpu.SemaphoreType.DMA((5,)),
            pltpu.SemaphoreType.DMA((NQ,)),
        ],
        compiler_params=pltpu.CompilerParams(vmem_limit_bytes=100 * 1024 * 1024),
        name="fused_block",
    )(A_x.reshape(S, D), A_wqkv, A_wo, B_w_gate, B_w_up, B_w_down)
    return out.reshape(1, S, D)
```

```python
import math

import jax
import jax.numpy as jnp
from jax import lax
import jax.experimental.pallas as pl
import jax.experimental.pallas.tpu as pltpu

S, D, H, DH, F = 2048, 512, 32, 16, 1376
TQ = 512
NQ = S // TQ
CK = 128
NC = S // CK
HG = 128 // DH
EPS = 1e-5
QSCALE = (DH ** -0.5) * math.log2(math.e)
L_LO, L_HI = 2.0 ** -60, 2.0 ** 60

NG = 18
LEAD = 6
DELAY = 20
CNT = [0] * NC
GROW = []
for _j in range(NG):
    _c = (_j * NC) // NG
    CNT[_c] += 1
    GROW.append(_c * CK + CK - 16 * CNT[_c])
NSTEP = NG * DH
NSLAB = NC * 8 - NG
NKF = (NG + DH - 1) // DH
KB_TICK = 2 * NG
KB_SRC = 2 * NG + 1

f32, bf16, u32 = jnp.float32, jnp.bfloat16, jnp.uint32
NT = (((1,), (1,)), ((), ()))
TN = (((0,), (0,)), ((), ()))


def _layernorm(x):
    m = jnp.mean(x, axis=-1, keepdims=True)
    xc = x - m
    v = jnp.mean(xc * xc, axis=-1, keepdims=True)
    return xc * lax.rsqrt(v + EPS)


def _gelu_tanh(x):
    c = math.sqrt(2.0 / math.pi)
    return 0.5 * x * (1.0 + jnp.tanh(c * (x + 0.044715 * (x * x * x))))


def _pack_pair(lo, hi):
    return pltpu.pack_elementwise([lo, hi], packed_dtype=bf16)


def _kernel(x_hbm, wqkv_hbm, wo_hbm, wg_hbm, wu_hbm, wd_hbm, out_hbm,
            x_s, wqkv_s, wo_s, wg_s, wu_s, wd_s, wqvt_s, k_s, kh_s, qt_s, qf_s, vt_s,
            kb_s, pbuf, lbuf, bad_s, sbuf, ot_s, h_s, hn_s, out_s, sem_x, sem_w, sem_o):
    def x_copy(i):
        return pltpu.make_async_copy(
            x_hbm.at[pl.ds(i * TQ, TQ), :], x_s.at[pl.ds(i * TQ, TQ), :], sem_x.at[i])

    def wqkv_copy(j):
        return pltpu.make_async_copy(
            wqkv_hbm.at[:, pl.ds(j * D, D)], wqkv_s.at[j], sem_w.at[j])

    def out_copy(i):
        return pltpu.make_async_copy(
            out_s.at[pl.ds(i * TQ, TQ), :], out_hbm.at[pl.ds(i * TQ, TQ), :], sem_o.at[i])

    late_copies = [
        pltpu.make_async_copy(src, dst, sem_w.at[3 + j])
        for j, (src, dst) in enumerate(
            [(wo_hbm, wo_s), (wg_hbm, wg_s), (wu_hbm, wu_s), (wd_hbm, wd_s)])
    ]
    x_copy(0).start()
    wqkv_copy(1).start()
    x_copy(1).start()
    wqkv_copy(0).start()
    wqkv_copy(2).start()
    x_copy(2).start()
    x_copy(3).start()

    def ln1(i):
        xu = pltpu.bitcast(x_s[pl.ds(i * TQ, TQ), :], u32)
        ne = _layernorm(pltpu.unpack_elementwise(xu, index=0, packed_dtype=bf16, unpacked_dtype=f32))
        no = _layernorm(pltpu.unpack_elementwise(xu, index=1, packed_dtype=bf16, unpacked_dtype=f32))
        xn = pltpu.bitcast(_pack_pair(ne, no), bf16)
        parts = []
        for a in range(TQ // 16):
            parts += [ne[a * 8:(a + 1) * 8], no[a * 8:(a + 1) * 8]]
        return xn, jnp.concatenate(parts, axis=0).astype(bf16)

    def proj_k(i, xp):
        kk = jnp.dot(xp, wqkv_s[1], preferred_element_type=f32).astype(bf16)
        ku = pltpu.bitcast(kk, u32)
        for g in range(D // 128):
            k_s[g, pl.ds(i * (TQ // 2), TQ // 2), :] = ku[:, g * 128:(g + 1) * 128]
        for j in range(NG):
            if GROW[j] // TQ == i:
                r0 = GROW[j] - i * TQ
                rows = kk[r0:r0 + 16].astype(f32)
                for g in range(D // 128):
                    kb_s[KB_SRC + g * NKF + j // DH, j % DH] = rows[:, g * 128:(g + 1) * 128]

    def proj_qv(i, xn):
        qv = lax.dot_general(wqvt_s[...], xn, NT, preferred_element_type=f32)
        pbuf[i] = pltpu.bitcast(qv, u32)
        q = qv[0:D] * QSCALE
        qt_s[i] = pltpu.bitcast(q.astype(bf16), u32).reshape(H, 8, TQ)
        for j in range(TQ // 128):
            qf_s[i, :, j * DH:(j + 1) * DH, :] = q[:, j * 128:(j + 1) * 128].reshape(H, DH, 128)
        vt_s[:, :, pl.ds(i * TQ, TQ)] = pltpu.bitcast(qv[D:2 * D].astype(bf16), u32).reshape(H, 8, TQ)

    x_copy(0).wait()
    xn0, xp0 = ln1(0)
    wqkv_copy(1).wait()
    x_copy(1).wait()
    proj_k(0, xp0)
    xn1, xp1 = ln1(1)
    wqkv_copy(0).wait()
    wqkv_copy(2).wait()
    proj_k(1, xp1)
    wqvt_s[0:D, :] = wqkv_s[0].T
    wqvt_s[D:2 * D, :] = wqkv_s[2].T
    x_copy(2).wait()
    x_copy(3).wait()
    for cp in late_copies:
        cp.start()
    proj_qv(0, xn0)
    xn2, xp2 = ln1(2)
    proj_k(2, xp2)
    xn3, xp3 = ln1(3)
    proj_qv(1, xn1)
    proj_k(3, xp3)
    proj_qv(2, xn2)
    proj_qv(3, xn3)
    lbuf[...] = jnp.ones(lbuf.shape, f32)
    bad_s[...] = jnp.zeros(bad_s.shape, f32)

    def shift_of(h):
        return (128 - (h % HG) * DH) % 128

    def kb_val(h, j, d, z):
        kk = kb_s[KB_SRC + (h // HG) * NKF + j // DH + z, j % DH]
        idx = jnp.full((16, 128), (h % HG) * DH + d, jnp.int32)
        return jnp.take_along_axis(kk, idx, axis=1, mode="promise_in_bounds")

    def make_kh(h, c, z):
        n = (CK - 16 * CNT[c]) // 2
        kh_s[pl.ds(c * 64, n), :] = pltpu.roll(k_s[h // HG + z, pl.ds(c * 64, n), :], shift_of(h), 1)

    def row_sum_inv(u):
        l = jnp.sum(lbuf[u], axis=0, keepdims=True)
        ok = jnp.logical_and(l >= L_LO, l <= L_HI)
        bad_s[u] = jnp.maximum(bad_s[u], jnp.where(ok, 0.0, 1.0))
        return 1.0 / l

    def pv_chunk(u, h, c):
        p = pltpu.bitcast(pbuf[u, pl.ds(c * 64, 64), :], bf16)
        v = pltpu.bitcast(vt_s[h, :, pl.ds(c * CK, CK)], bf16)
        return jnp.dot(v, p, preferred_element_type=f32)

    def block(h, carry):
        h_prep = jnp.minimum(h + 1, H - 1)
        h_prev = jnp.maximum(h - 1, 0)
        hrow = pl.multiple_of(h_prev * DH, DH)
        slot = h % 2
        z = lax.shift_right_logical(h, 20)
        lpart = [None] * NQ
        loaded = set()
        st = dict(a2=None, step=0, slab=0, prod=0)
        queue = []

        def emit(u, row0, s16):
            p = jnp.exp2(s16)
            pair = p[0:8] + p[8:16]
            lpart[u] = pair if lpart[u] is None else lpart[u] + pair
            pbuf[u, pl.ds(row0 // 2, 8), :] = _pack_pair(p[0:8], p[8:16])

        def flush(gn):
            while queue and queue[0][0] <= gn:
                _, jj, dd, val = queue.pop(0)
                kb_s[(1 - slot) * NG + jj, dd] = val

        def vpu_step():
            gn = st["step"]
            st["step"] += 1
            u, n = divmod(gn, NSTEP)
            j, d = divmod(n, DH)
            kb = kb_s[slot * NG + j + z, d]
            qb = jnp.concatenate(
                [qf_s[u, h, pl.ds(jj * DH + d, 8, stride=0), :] for jj in range(4)], axis=1)
            t = jnp.concatenate([kb] * 4, axis=1).reshape(2, 8, TQ) * qb[None]
            st["a2"] = t if d == 0 else st["a2"] + t
            if d == DH - 1:
                assert (u, GROW[j] // CK) in loaded
                emit(u, GROW[j], st["a2"].reshape(16, TQ))
            if gn % NQ == 0:
                dd, jj = divmod(st["prod"], NG)
                st["prod"] += 1
                queue.append((gn + DELAY, jj, dd, kb_val(h_prep, jj, dd, z)))
            if gn == NQ * NSTEP - 1:
                flush(10 ** 9)

        def due(half):
            return (st["step"] < NQ * NSTEP
                    and st["step"] * NSLAB * 2 < (st["slab"] * 2 + half + LEAD) * NSTEP)

        for u in range(NQ):
            linv = row_sum_inv(u)
            w = pltpu.bitcast(qt_s[u, h], bf16)
            for c in range(NC):
                nr = CK - 16 * CNT[c]
                kc = pltpu.bitcast(kh_s[pl.ds(c * 64, nr // 2), :], bf16)
                s = jnp.dot(kc[:, 0:DH], w, preferred_element_type=f32)
                if u == NQ - 1:
                    make_kh(h_prep, c, z)
                pv = pv_chunk(u, h_prev, c)
                loaded.add((u, c))
                acc = pv if c == 0 else pv + acc
                if u == 0 and c == 0:
                    while due(0):
                        vpu_step()
                for r in range(nr // 16):
                    s16 = s[r * 16:(r + 1) * 16, :]
                    if r == 0 and (NQ - 2, NC - 2) <= (u, c) < (NQ - 1, NC - 2):
                        k_s[D // 128, 0:8, :] = pltpu.bitcast(s16[0:8, 0:128], u32)
                    if due(1):
                        flush(st["step"])
                        kb_s[KB_TICK, 0, 0:8, :] = s16[0:8, 0:128]
                        while due(1):
                            vpu_step()
                    emit(u, c * CK + r * 16, s16)
                    st["slab"] += 1
            ot_s[u, pl.ds(hrow, DH), :] = (acc * linv).astype(bf16)
            lbuf[u] = lpart[u]
        return carry

    for d in range(DH):
        for j in range(NG):
            kb_s[j, d] = kb_val(0, j, d, 0)
    for c in range(NC):
        make_kh(0, c, 0)
    lax.fori_loop(0, H, block, 0)

    for u in range(NQ):
        row_sum_inv(u)
    n_bad = jnp.max(bad_s[...])

    @pl.when(n_bad > 0.0)
    def _():
        def one(t, carry):
            h = t // NQ
            u = t % NQ
            hrow = pl.multiple_of(h * DH, DH)
            w = pltpu.bitcast(qt_s[u, h], bf16)

            def scores(c, m):
                r0 = pl.multiple_of(c * 64, 64)
                kc = pltpu.roll(k_s[h // HG, pl.ds(r0, 64), :], shift_of(h), 1)
                s = jnp.dot(pltpu.bitcast(kc, bf16)[:, 0:DH], w, preferred_element_type=f32)
                sbuf[c] = s
                return jnp.maximum(m, jnp.max(s, axis=0, keepdims=True))

            m = lax.fori_loop(0, NC, scores, jnp.full((1, TQ), -jnp.inf, f32))

            def probs(c, l):
                p = jnp.exp2(sbuf[c] - m)
                for r in range(CK // 16):
                    lo, hi = p[r * 16:r * 16 + 8], p[r * 16 + 8:r * 16 + 16]
                    l = l + (lo + hi)
                    pbuf[u, pl.ds(pl.multiple_of(c * 64 + r * 8, 8), 8), :] = _pack_pair(lo, hi)
                return l

            l = lax.fori_loop(0, NC, probs, jnp.zeros((8, TQ), f32))
            lbuf[u] = l
            acc = pv_chunk(u, h, 0)
            for c in range(1, NC):
                acc = pv_chunk(u, h, c) + acc
            linv = 1.0 / jnp.sum(l, axis=0, keepdims=True)
            ot_s[u, pl.ds(hrow, DH), :] = (acc * linv).astype(bf16)
            return carry

        lax.fori_loop(0, H * NQ, one, 0)

    for cp in late_copies:
        cp.wait()
    for u in range(NQ):
        hrow = (H - 1) * DH
        linv = 1.0 / jnp.sum(lbuf[u], axis=0, keepdims=True)
        acc = pv_chunk(u, H - 1, 0)
        for c in range(1, NC):
            acc = pv_chunk(u, H - 1, c) + acc
        ot_s[u, pl.ds(hrow, DH), :] = (acc * linv).astype(bf16)
    for u in range(NQ):
        attn = lax.dot_general(ot_s[u], wo_s[...], TN, preferred_element_type=f32)
        h = x_s[pl.ds(u * TQ, TQ), :].astype(f32) + attn
        h_s[u] = h
        hn_s[u] = _layernorm(h).astype(bf16)

    def ffn(i, carry):
        rows = pl.ds(pl.multiple_of(i * TQ, TQ), TQ)
        hn = hn_s[i]
        gate = lax.dot_general(hn, wg_s[...], NT, preferred_element_type=f32)
        up = lax.dot_general(hn, wu_s[...], NT, preferred_element_type=f32)
        act = (_gelu_tanh(gate) * up).astype(bf16)
        y = h_s[i] + jnp.dot(act, wd_s[...], preferred_element_type=f32)
        out_s[rows, :] = y.astype(bf16)
        out_copy(i).start()
        return carry

    lax.fori_loop(0, NQ, ffn, 0)
    for i in range(NQ):
        out_copy(i).wait()


@jax.jit
def pallas_sequential_preLN__softmax_full_mha__geglu_ffn__prompt_kernel(
    A_x: jax.Array,
    A_wqkv: jax.Array,
    A_wo: jax.Array,
    B_x: jax.Array,
    B_w_gate: jax.Array,
    B_w_up: jax.Array,
    B_w_down: jax.Array,
):
    del B_x
    hbm_spec = pl.BlockSpec(memory_space=pltpu.HBM)
    out = pl.pallas_call(
        _kernel,
        out_shape=jax.ShapeDtypeStruct((S, D), bf16),
        in_specs=[hbm_spec] * 6,
        out_specs=hbm_spec,
        scratch_shapes=[
            pltpu.VMEM((S, D), bf16),
            pltpu.VMEM((3, D, D), bf16),
            pltpu.VMEM((D, D), bf16),
            pltpu.VMEM((F, D), bf16),
            pltpu.VMEM((F, D), bf16),
            pltpu.VMEM((F, D), bf16),
            pltpu.VMEM((2 * D, D), bf16),
            pltpu.VMEM((D // 128 + 1, S // 2, 128), u32),
            pltpu.VMEM((S // 2, 128), u32),
            pltpu.VMEM((NQ, H, 8, TQ), u32),
            pltpu.VMEM((NQ, H, 4 * DH, 128), f32),
            pltpu.VMEM((H, 8, S), u32),
            pltpu.VMEM((KB_SRC + 4 * NKF, DH, 16, 128), f32),
            pltpu.VMEM((NQ, S // 2, TQ), u32),
            pltpu.VMEM((NQ, 8, TQ), f32),
            pltpu.VMEM((NQ, 1, TQ), f32),
            pltpu.VMEM((NC, CK, TQ), f32),
            pltpu.VMEM((NQ, D, TQ), bf16),
            pltpu.VMEM((NQ, TQ, D), f32),
            pltpu.VMEM((NQ, TQ, D), bf16),
            pltpu.VMEM((S, D), bf16),
            pltpu.SemaphoreType.DMA((NQ,)),
            pltpu.SemaphoreType.DMA((7,)),
            pltpu.SemaphoreType.DMA((NQ,)),
        ],
        compiler_params=pltpu.CompilerParams(vmem_limit_bytes=100 * 1024 * 1024),
        name="fused_block",
    )(A_x.reshape(S, D), A_wqkv, A_wo, B_w_gate.T, B_w_up.T, B_w_down)
    return out.reshape(1, S, D)
```

```python
import math

import jax
import jax.numpy as jnp
from jax import lax
import jax.experimental.pallas as pl
import jax.experimental.pallas.tpu as pltpu

S, D, H, DH, F = 2048, 512, 32, 16, 1376
TQ = 512
NQ = S // TQ
CK = 128
NC = S // CK
HG = 128 // DH
NO = 2
EPS = 1e-5
QSCALE = (DH ** -0.5) * math.log2(math.e)
L_LO, L_HI = 2.0 ** -60, 2.0 ** 60

NG = 18
LEAD = 10
LNLAG = 5
PVLEAD = 6
DELAY = 20
CNT = [0] * NC
GROW = []
for _j in range(NG):
    _c = max(0, (_j * NC) // NG - 1)
    CNT[_c] += 1
    GROW.append(_c * CK + CK - 16 * CNT[_c])
NSTEP = NG * DH
NSLAB = NC * 8 - NG
NKF = (NG + DH - 1) // DH
KB_TICK = 2 * NG
KB_SRC = 2 * NG + 1

f32, bf16, u32 = jnp.float32, jnp.bfloat16, jnp.uint32
NT = (((1,), (1,)), ((), ()))
TN = (((0,), (0,)), ((), ()))


def _layernorm(x):
    m = jnp.mean(x, axis=-1, keepdims=True)
    xc = x - m
    v = jnp.mean(xc * xc, axis=-1, keepdims=True)
    return xc * lax.rsqrt(v + EPS)


def _gelu_tanh(x):
    c = math.sqrt(2.0 / math.pi)
    return 0.5 * x * (1.0 + jnp.tanh(c * (x + 0.044715 * (x * x * x))))


def _pack(x):
    return pltpu.bitcast(x.astype(bf16), u32)


def _kernel(x_hbm, wqkv_hbm, wo_hbm, wg_hbm, wu_hbm, wd_hbm, out_hbm,
            x_s, wqkv_s, wg_s, wu_s, wd_s, wqvt_s, k_s, kh_s, qt_s, qf_s, vt_s,
            kb_s, pbuf, lbuf, bad_s, sbuf, ot_s, h_s, hn_s, out_s, sem_x, sem_w, sem_o):
    def x_copy(i):
        return pltpu.make_async_copy(
            x_hbm.at[pl.ds(i * TQ, TQ), :], x_s.at[pl.ds(i * TQ, TQ), :], sem_x.at[i])

    def wqkv_copy(j):
        return pltpu.make_async_copy(
            wqkv_hbm.at[:, pl.ds(j * D, D)], wqkv_s.at[j], sem_w.at[j])

    def out_copy(i, j):
        rows, cols = pl.ds(i * TQ, TQ), pl.ds(j * (D // NO), D // NO)
        return pltpu.make_async_copy(
            out_s.at[rows, cols], out_hbm.at[rows, cols], sem_o.at[i * NO + j])

    late_copies = [
        pltpu.make_async_copy(src, dst, sem_w.at[3 + j])
        for j, (src, dst) in enumerate(
            [(wo_hbm, hn_s.at[NQ]), (wg_hbm, wg_s), (wu_hbm, wu_s), (wd_hbm, wd_s)])
    ]
    x_copy(0).start()
    wqkv_copy(1).start()
    for i in range(1, NQ):
        x_copy(i).start()
    wqkv_copy(0).start()
    wqkv_copy(2).start()

    def ln1(i):
        return _layernorm(x_s[pl.ds(i * TQ, TQ), :].astype(f32)).astype(bf16)

    def proj_k(row0, xn):
        n = xn.shape[0]
        kk = jnp.dot(xn, wqkv_s[1], preferred_element_type=f32)
        for g in range(D // 128):
            k_s[pl.ds(g * (S // 2) + row0 // 2, n // 2), :] = _pack(kk[:, g * 128:(g + 1) * 128])
        for j in range(NG):
            r0 = GROW[j] - row0
            if 0 <= r0 < n:
                for g in range(D // 128):
                    kb_s[KB_SRC + g * NKF + j // DH, j % DH] = kk[r0:r0 + 16, g * 128:(g + 1) * 128]

    def proj_qv(i, xn):
        qv = lax.dot_general(wqvt_s[...], xn, NT, preferred_element_type=f32)
        pbuf[pl.ds(i * (S // 2), S // 2), :] = pltpu.bitcast(qv, u32)
        q = qv[0:D] * QSCALE
        qt_s[pl.ds(i * (D // 2), D // 2), :] = _pack(q)
        for j in range(TQ // 128):
            qf_s[i, :, j * DH:(j + 1) * DH, :] = q[:, j * 128:(j + 1) * 128].reshape(H, DH, 128)
        vt_s[:, pl.ds(i * TQ, TQ)] = _pack(qv[D:2 * D])

    HT = TQ // 2
    x_copy(0).wait()
    xn0 = ln1(0)
    wqkv_copy(1).wait()
    proj_k(0, xn0[:HT])
    x_copy(1).wait()
    proj_k(HT, xn0[HT:])
    xn1 = ln1(1)
    proj_k(TQ, xn1[:HT])
    x_copy(2).wait()
    proj_k(TQ + HT, xn1[HT:])
    xn2 = ln1(2)
    proj_k(2 * TQ, xn2[:HT])
    x_copy(3).wait()
    wqkv_copy(0).wait()
    wqkv_copy(2).wait()
    for cp in late_copies:
        cp.start()
    proj_k(2 * TQ + HT, xn2[HT:])
    xn3 = ln1(3)
    proj_k(3 * TQ, xn3)
    wqvt_s[0:D, :] = wqkv_s[0].T
    wqvt_s[D:2 * D, :] = wqkv_s[2].T
    for i, xn in enumerate((xn0, xn1, xn2, xn3)):
        proj_qv(i, xn)
    lbuf[...] = jnp.ones(lbuf.shape, f32)
    bad_s[...] = jnp.zeros(bad_s.shape, f32)

    def aligned(v, n):
        return v if isinstance(v, int) else pl.multiple_of(v, n)

    def q_weights(u, h):
        return pltpu.bitcast(qt_s[pl.ds(aligned(u * (D // 2) + h * 8, 8), 8), :], bf16)

    def shift_of(h):
        return (128 - (h % HG) * DH) % 128

    def kb_val(h, j, d, z):
        kk = kb_s[KB_SRC + (h // HG) * NKF + j // DH + z, j % DH]
        idx = jnp.full((16, 128), (h % HG) * DH + d, jnp.int32)
        return jnp.take_along_axis(kk, idx, axis=1, mode="promise_in_bounds")

    def make_kh(h, c, z):
        n = (CK - 16 * CNT[c]) // 2
        kh_s[pl.ds(c * 64, n), :] = pltpu.roll(
            k_s[pl.ds(aligned((h // HG + z) * (S // 2), S // 2) + c * 64, n), :], shift_of(h), 1)

    def row_sum_inv(u):
        l = jnp.sum(lbuf[u], axis=0, keepdims=True)
        ok = jnp.logical_and(l >= L_LO, l <= L_HI)
        bad_s[u] = jnp.maximum(bad_s[u], jnp.where(ok, 0.0, 1.0))
        return 1.0 / l

    def pv_chunk(u, h, c):
        p = pltpu.bitcast(pbuf[pl.ds(aligned(u * (S // 2), 64) + c * 64, 64), :], bf16)
        v = pltpu.bitcast(vt_s[pl.ds(aligned(h * 8, 8), 8), pl.ds(c * CK, CK)], bf16)
        return jnp.dot(v, p, preferred_element_type=f32)

    def block(h, carry):
        h_prep = jnp.minimum(h + 1, H - 1)
        h_prev = jnp.maximum(h - 1, 0)
        hrow = pl.multiple_of(h_prev * DH, DH)
        slot = h % 2
        z = lax.shift_right_logical(h, 20)
        lpart = [None] * NQ
        loaded = set()
        st = dict(a2=None, step=0, slab=0, prod=0)
        queue = []

        def emit(u, row0, s16):
            p = jnp.exp2(s16)
            pair = p[0:8] + p[8:16]
            lpart[u] = pair if lpart[u] is None else lpart[u] + pair
            pbuf[pl.ds(u * (S // 2) + row0 // 2, 8), :] = _pack(p)

        def flush(gn):
            while queue and queue[0][0] <= gn:
                _, jj, dd, val = queue.pop(0)
                kb_s[(1 - slot) * NG + jj, dd] = val

        def vpu_step():
            gn = st["step"]
            st["step"] += 1
            u, n = divmod(gn, NSTEP)
            j, d = divmod(n, DH)
            kb = kb_s[slot * NG + j + z, d]
            qb = jnp.concatenate(
                [qf_s[u, h, pl.ds(jj * DH + d, 8, stride=0), :] for jj in range(4)], axis=1)
            t = jnp.concatenate([kb] * 4, axis=1).reshape(2, 8, TQ) * qb[None]
            st["a2"] = t if d == 0 else st["a2"] + t
            if d == DH - 1:
                assert (u, GROW[j] // CK) in loaded
                emit(u, GROW[j], st["a2"].reshape(16, TQ))
            if gn % NQ == 0:
                dd, jj = divmod(st["prod"], NG)
                st["prod"] += 1
                queue.append((gn + DELAY, jj, dd, kb_val(h_prep, jj, dd, z)))
            if gn == NQ * NSTEP - 1:
                flush(10 ** 9)

        def due(half):
            return (st["step"] < NQ * NSTEP
                    and st["step"] * NSLAB * 2 < (st["slab"] * 2 + half + LEAD) * NSTEP)

        for u in range(NQ):
            linv = row_sum_inv(u)
            w = q_weights(u, h)
            for c in range(NC):
                nr = CK - 16 * CNT[c]
                kc = pltpu.bitcast(kh_s[pl.ds(c * 64, nr // 2), :], bf16)
                s = jnp.dot(kc[:, 0:DH], w, preferred_element_type=f32)
                if u == NQ - 1:
                    make_kh(h_prep, c, z)
                pv = pv_chunk(u, h_prev, c)
                loaded.add((u, c))
                acc = pv if c == 0 else pv + acc
                if u == 0 and c == 0:
                    while due(0):
                        vpu_step()
                for r in range(nr // 16):
                    s16 = s[r * 16:(r + 1) * 16, :]
                    if r == 0 and (NQ - 2, NC - 2) <= (u, c) < (NQ - 1, NC - 2):
                        k_s[pl.ds((D // 128) * (S // 2), 8), :] = pltpu.bitcast(s16[0:8, 0:128], u32)
                    if due(1):
                        flush(st["step"])
                        kb_s[KB_TICK, 0, 0:8, :] = s16[0:8, 0:128]
                        while due(1):
                            vpu_step()
                    emit(u, c * CK + r * 16, s16)
                    st["slab"] += 1
            ot_s[u, pl.ds(hrow, DH), :] = (acc * linv).astype(bf16)
            lbuf[u] = lpart[u]
        return carry + h

    for d in range(DH):
        for j in range(NG):
            kb_s[j, d] = kb_val(0, j, d, 0)
    for c in range(NC):
        make_kh(0, c, 0)
    cnt = lax.fori_loop(0, H, block, jnp.int32(0))

    for u in range(NQ):
        row_sum_inv(u)
    n_bad = jnp.max(bad_s[...])

    @pl.when(n_bad > 0.0)
    def _():
        def one(t, carry):
            h = t // NQ
            u = t % NQ
            hrow = pl.multiple_of(h * DH, DH)
            w = q_weights(u, h)

            def scores(c, m):
                r0 = pl.multiple_of((h // HG) * (S // 2) + c * 64, 64)
                kc = pltpu.roll(k_s[pl.ds(r0, 64), :], shift_of(h), 1)
                s = jnp.dot(pltpu.bitcast(kc, bf16)[:, 0:DH], w, preferred_element_type=f32)
                sbuf[c] = s
                return jnp.maximum(m, jnp.max(s, axis=0, keepdims=True))

            m = lax.fori_loop(0, NC, scores, jnp.full((1, TQ), -jnp.inf, f32))

            def probs(c, l):
                p = jnp.exp2(sbuf[c] - m)
                pbuf[pl.ds(pl.multiple_of(u * (S // 2) + c * 64, 64), 64), :] = _pack(p)
                return l + jnp.sum(p.reshape(CK // 8, 8, TQ), axis=0)

            l = lax.fori_loop(0, NC, probs, jnp.zeros((8, TQ), f32))
            lbuf[u] = l
            acc = pv_chunk(u, h, 0)
            for c in range(1, NC):
                acc = pv_chunk(u, h, c) + acc
            linv = 1.0 / jnp.sum(l, axis=0, keepdims=True)
            ot_s[u, pl.ds(hrow, DH), :] = (acc * linv).astype(bf16)
            return carry

        lax.fori_loop(0, H * NQ, one, 0)

    for cp in late_copies:
        cp.wait()
    NB = TQ // 128
    wo_v = hn_s.at[NQ + lax.shift_right_logical(cnt, 20)]
    pending = []

    def finish(now):
        while pending and pending[0][0] <= now:
            _, t, rb, y = pending.pop(0)
            rows = slice(rb * 128, (rb + 1) * 128)
            h = x_s[pl.ds(t * TQ + rb * 128, 128), :].astype(f32) + y
            h_s[t, rows, :] = h
            hn_s[t, rows, :] = _layernorm(h).astype(bf16)

    pv_state = dict(n=0, acc=None)

    def last_pv(upto):
        while pv_state["n"] < min(upto, NQ * NC):
            u, c = divmod(pv_state["n"], NC)
            pv_state["n"] += 1
            pv = pv_chunk(u, H - 1, c)
            pv_state["acc"] = pv if c == 0 else pv + pv_state["acc"]
            if c == NC - 1:
                linv = 1.0 / jnp.sum(lbuf[u], axis=0, keepdims=True)
                ot_s[u, pl.ds((H - 1) * DH, DH), :] = (pv_state["acc"] * linv).astype(bf16)

    last_pv(NC + PVLEAD)
    for u in range(NQ):
        o_nat = ot_s[u].T
        cols = []
        for c in range(NC):
            n = u * NC + c
            finish(n)
            rb, nt = divmod(c, NB)
            cols.append(jnp.dot(o_nat[rb * 128:(rb + 1) * 128], wo_v[:, nt * 128:(nt + 1) * 128],
                                preferred_element_type=f32))
            last_pv(NC + PVLEAD + n + 1)
            if len(cols) == NB:
                pending.append((n + LNLAG, u, rb, jnp.concatenate(cols, axis=1)))
                cols = []
    finish(10 ** 9)

    def ffn(i, carry):
        rows = pl.ds(aligned(i * TQ, TQ), TQ)
        hn = hn_s[i]
        gate_t = lax.dot_general(wg_s[...], hn, NT, preferred_element_type=f32)
        up_t = lax.dot_general(wu_s[...], hn, NT, preferred_element_type=f32)
        act = (_gelu_tanh(gate_t) * up_t).astype(bf16).T
        for j in range(NO):
            cols = slice(j * (D // NO), (j + 1) * (D // NO))
            y = h_s[i, :, cols] + jnp.dot(act, wd_s[:, cols], preferred_element_type=f32)
            out_s[rows, cols] = y.astype(bf16)
            out_copy(i, j).start()
        return carry

    lax.fori_loop(0, NQ, ffn, 0)
    for i in range(NQ):
        for j in range(NO):
            out_copy(i, j).wait()


@jax.jit
def pallas_sequential_preLN__softmax_full_mha__geglu_ffn__prompt_kernel(
    A_x: jax.Array,
    A_wqkv: jax.Array,
    A_wo: jax.Array,
    B_x: jax.Array,
    B_w_gate: jax.Array,
    B_w_up: jax.Array,
    B_w_down: jax.Array,
):
    del B_x
    hbm_spec = pl.BlockSpec(memory_space=pltpu.HBM)
    out = pl.pallas_call(
        _kernel,
        out_shape=jax.ShapeDtypeStruct((S, D), bf16),
        in_specs=[hbm_spec] * 6,
        out_specs=hbm_spec,
        scratch_shapes=[
            pltpu.VMEM((S, D), bf16),
            pltpu.VMEM((3, D, D), bf16),
            pltpu.VMEM((F, D), bf16),
            pltpu.VMEM((F, D), bf16),
            pltpu.VMEM((F, D), bf16),
            pltpu.VMEM((2 * D, D), bf16),
            pltpu.VMEM(((D // 128) * (S // 2) + 32, 128), u32),
            pltpu.VMEM((S // 2, 128), u32),
            pltpu.VMEM((NQ * D // 2, TQ), u32),
            pltpu.VMEM((NQ, H, 4 * DH, 128), f32),
            pltpu.VMEM((D // 2, S), u32),
            pltpu.VMEM((KB_SRC + 4 * NKF, DH, 16, 128), f32),
            pltpu.VMEM((NQ * S // 2, TQ), u32),
            pltpu.VMEM((NQ, 8, TQ), f32),
            pltpu.VMEM((NQ, 8, TQ), f32),
            pltpu.VMEM((NC, CK, TQ), f32),
            pltpu.VMEM((NQ, D, TQ), bf16),
            pltpu.VMEM((NQ, TQ, D), f32),
            pltpu.VMEM((NQ + 1, TQ, D), bf16),
            pltpu.VMEM((S, D), bf16),
            pltpu.SemaphoreType.DMA((NQ,)),
            pltpu.SemaphoreType.DMA((7,)),
            pltpu.SemaphoreType.DMA((NQ * NO,)),
        ],
        compiler_params=pltpu.CompilerParams(vmem_limit_bytes=100 * 1024 * 1024),
        name="fused_block",
    )(A_x.reshape(S, D), A_wqkv, A_wo, B_w_gate.T, B_w_up.T, B_w_down)
    return out.reshape(1, S, D)
```

```python
import math

import jax
import jax.numpy as jnp
from jax import lax
import jax.experimental.pallas as pl
import jax.experimental.pallas.tpu as pltpu

S, D, H, DH, F = 2048, 512, 32, 16, 1376
TQ = 512
NQ = S // TQ
CK = 128
NC = S // CK
HG = 128 // DH
NO = 2
EPS = 1e-5
QSCALE = (DH ** -0.5) * math.log2(math.e)
L_LO, L_HI = 2.0 ** -60, 2.0 ** 60

NG = 18
LEAD = 10
LNLAG = 5
PVLEAD = 6
DELAY = 18
CNT = [0] * NC
GROW = []
for _j in range(NG):
    _c = max(0, (_j * NC) // NG - 1)
    CNT[_c] += 1
    GROW.append(_c * CK + CK - 16 * CNT[_c])
NSTEP = NG * DH
NSLAB = NC * 8 - NG
NKF = (NG + DH - 1) // DH
KB_TICK = 2 * NG
KB_SRC = 2 * NG + 1

f32, bf16, u32 = jnp.float32, jnp.bfloat16, jnp.uint32
NT = (((1,), (1,)), ((), ()))
TN = (((0,), (0,)), ((), ()))


def _layernorm(x):
    m = jnp.mean(x, axis=-1, keepdims=True)
    xc = x - m
    v = jnp.mean(xc * xc, axis=-1, keepdims=True)
    return xc * lax.rsqrt(v + EPS)


def _gelu_tanh(x):
    c = math.sqrt(2.0 / math.pi)
    return 0.5 * x * (1.0 + jnp.tanh(c * (x + 0.044715 * (x * x * x))))


def _pack(x):
    return pltpu.bitcast(x.astype(bf16), u32)


def _kernel(x_hbm, wqkv_hbm, wo_hbm, wg_hbm, wu_hbm, wd_hbm, out_hbm,
            x_s, wqkv_s, wg_s, wu_s, wd_s, wqvt_s, k_s, kh_s, qt_s, qf_s, vt_s,
            kb_s, pbuf, lbuf, bad_s, sbuf, ot_s, h_s, hn_s, out_s, sem_x, sem_w, sem_o):
    def x_copy(i):
        return pltpu.make_async_copy(
            x_hbm.at[pl.ds(i * TQ, TQ), :], x_s.at[pl.ds(i * TQ, TQ), :], sem_x.at[i])

    def wqkv_copy(j):
        return pltpu.make_async_copy(
            wqkv_hbm.at[:, pl.ds(j * D, D)], wqkv_s.at[j], sem_w.at[j])

    def out_copy(i, j):
        rows, cols = pl.ds(i * TQ, TQ), pl.ds(j * (D // NO), D // NO)
        return pltpu.make_async_copy(
            out_s.at[rows, cols], out_hbm.at[rows, cols], sem_o.at[i * NO + j])

    late_copies = [
        pltpu.make_async_copy(src, dst, sem_w.at[3 + j])
        for j, (src, dst) in enumerate(
            [(wo_hbm, hn_s.at[NQ]), (wg_hbm, wg_s), (wu_hbm, wu_s), (wd_hbm, wd_s)])
    ]
    x_copy(0).start()
    wqkv_copy(1).start()
    for i in range(1, NQ):
        x_copy(i).start()
    wqkv_copy(0).start()
    wqkv_copy(2).start()

    def ln1(i):
        return _layernorm(x_s[pl.ds(i * TQ, TQ), :].astype(f32)).astype(bf16)

    def proj_k(row0, xn):
        n = xn.shape[0]
        kk = jnp.dot(xn, wqkv_s[1], preferred_element_type=f32)
        for g in range(D // 128):
            k_s[pl.ds(g * (S // 2) + row0 // 2, n // 2), :] = _pack(kk[:, g * 128:(g + 1) * 128])
        for j in range(NG):
            r0 = GROW[j] - row0
            if 0 <= r0 < n:
                for g in range(D // 128):
                    kb_s[KB_SRC + g * NKF + j // DH, j % DH] = kk[r0:r0 + 16, g * 128:(g + 1) * 128]

    def proj_qv(i, xn):
        qv = lax.dot_general(wqvt_s[...], xn, NT, preferred_element_type=f32)
        pbuf[pl.ds(i * (S // 2), S // 2), :] = pltpu.bitcast(qv, u32)
        for h in range(H):
            q = qv[2 * DH * h:2 * DH * h + DH] * QSCALE
            qt_s[pl.ds(i * (D // 2) + h * 8, 8), :] = _pack(q)
            for d in range(DH):
                qf_s[i, h, d] = jnp.broadcast_to(q[d:d + 1], (8, TQ))
            vt_s[pl.ds(h * 8, 8), pl.ds(i * TQ, TQ)] = _pack(qv[2 * DH * h + DH:2 * DH * (h + 1)])

    HT = TQ // 2
    x_copy(0).wait()
    xn0 = ln1(0)
    wqkv_copy(1).wait()
    proj_k(0, xn0[:HT])
    x_copy(1).wait()
    proj_k(HT, xn0[HT:])
    xn1 = ln1(1)
    proj_k(TQ, xn1[:HT])
    x_copy(2).wait()
    proj_k(TQ + HT, xn1[HT:])
    xn2 = ln1(2)
    proj_k(2 * TQ, xn2[:HT])
    x_copy(3).wait()
    wqkv_copy(0).wait()
    wqkv_copy(2).wait()
    for cp in late_copies:
        cp.start()
    proj_k(2 * TQ + HT, xn2[HT:])
    xn3 = ln1(3)
    proj_k(3 * TQ, xn3)
    wq_t, wv_t = wqkv_s[0].T, wqkv_s[2].T
    for h in range(H):
        wqvt_s[2 * DH * h:2 * DH * h + DH, :] = wq_t[h * DH:(h + 1) * DH]
        wqvt_s[2 * DH * h + DH:2 * DH * (h + 1), :] = wv_t[h * DH:(h + 1) * DH]
    for i, xn in enumerate((xn0, xn1, xn2, xn3)):
        proj_qv(i, xn)
    lbuf[...] = jnp.ones(lbuf.shape, f32)
    bad_s[...] = jnp.zeros(bad_s.shape, f32)

    def aligned(v, n):
        return v if isinstance(v, int) else pl.multiple_of(v, n)

    def q_weights(u, h):
        return pltpu.bitcast(qt_s[pl.ds(aligned(u * (D // 2) + h * 8, 8), 8), :], bf16)

    def shift_of(h):
        return (128 - (h % HG) * DH) % 128

    def kb_val(h, j, d, z):
        kk = kb_s[KB_SRC + (h // HG) * NKF + j // DH + z, j % DH]
        idx = jnp.full((16, 128), (h % HG) * DH + d, jnp.int32)
        return jnp.take_along_axis(kk, idx, axis=1, mode="promise_in_bounds")

    def make_kh(h, c, z):
        n = (CK - 16 * CNT[c]) // 2
        kh_s[pl.ds(c * 64, n), :] = pltpu.roll(
            k_s[pl.ds(aligned((h // HG + z) * (S // 2), S // 2) + c * 64, n), :], shift_of(h), 1)

    def row_sum_inv(u):
        l = jnp.sum(lbuf[u], axis=0, keepdims=True)
        ok = jnp.logical_and(l >= L_LO, l <= L_HI)
        bad_s[u] = jnp.maximum(bad_s[u], jnp.where(ok, 0.0, 1.0))
        return 1.0 / l

    def pv_chunk(u, h, c):
        p = pltpu.bitcast(pbuf[pl.ds(aligned(u * (S // 2), 64) + c * 64, 64), :], bf16)
        v = pltpu.bitcast(vt_s[pl.ds(aligned(h * 8, 8), 8), pl.ds(c * CK, CK)], bf16)
        return jnp.dot(v, p, preferred_element_type=f32)

    def block(h, carry):
        h_prep = jnp.minimum(h + 1, H - 1)
        h_prev = jnp.maximum(h - 1, 0)
        hrow = pl.multiple_of(h_prev * DH, DH)
        slot = h % 2
        z = lax.shift_right_logical(h, 20)
        lpart = [None] * NQ
        loaded = set()
        st = dict(a2=None, step=0, slab=0, prod=0)
        queue = []

        def emit(u, row0, s16):
            p = jnp.exp2(s16)
            pair = p[0:8] + p[8:16]
            lpart[u] = pair if lpart[u] is None else lpart[u] + pair
            pbuf[pl.ds(u * (S // 2) + row0 // 2, 8), :] = _pack(p)

        def flush(gn):
            while queue and queue[0][0] <= gn:
                _, jj, dd, val = queue.pop(0)
                kb_s[(1 - slot) * NG + jj, dd] = val

        def vpu_steps(target):
            while st["step"] < target:
                g0 = st["step"]
                u, n = divmod(g0, NSTEP)
                j, d0 = divmod(n, DH)
                cnt = min(target - g0, DH - d0)
                st["step"] += cnt
                kb = kb_s[slot * NG + j + z, d0:d0 + cnt]
                kb = jnp.concatenate([kb] * 4, axis=2).reshape(cnt, 2, 8, TQ)
                t = kb * qf_s[u, h, d0:d0 + cnt][:, None]
                for i in range(cnt):
                    st["a2"] = t[i] if d0 + i == 0 else st["a2"] + t[i]
                if d0 + cnt == DH:
                    assert (u, GROW[j] // CK) in loaded
                    emit(u, GROW[j], st["a2"].reshape(16, TQ))
                while st["prod"] * NQ < st["step"]:
                    dd, jj = divmod(st["prod"], NG)
                    queue.append((st["prod"] * NQ + DELAY, jj, dd, kb_val(h_prep, jj, dd, z)))
                    st["prod"] += 1
            if st["step"] == NQ * NSTEP:
                flush(10 ** 9)

        def due(half):
            num = (st["slab"] * 2 + half + LEAD) * NSTEP
            return min(NQ * NSTEP, -(-num // (2 * NSLAB)))

        for u in range(NQ):
            linv = row_sum_inv(u)
            w = q_weights(u, h)
            for c in range(NC):
                nr = CK - 16 * CNT[c]
                kc = pltpu.bitcast(kh_s[pl.ds(c * 64, nr // 2), :], bf16)
                s = jnp.dot(kc[:, 0:DH], w, preferred_element_type=f32)
                if u == NQ - 1:
                    make_kh(h_prep, c, z)
                pv = pv_chunk(u, h_prev, c)
                loaded.add((u, c))
                acc = pv if c == 0 else pv + acc
                if u == 0 and c == 0:
                    vpu_steps(due(0))
                for r in range(nr // 16):
                    s16 = s[r * 16:(r + 1) * 16, :]
                    if r == 0 and (NQ - 2, NC - 2) <= (u, c) < (NQ - 1, NC - 2):
                        k_s[pl.ds((D // 128) * (S // 2), 8), :] = pltpu.bitcast(s16[0:8, 0:128], u32)
                    if st["step"] < due(1):
                        flush(st["step"])
                        kb_s[KB_TICK, 0, 0:8, :] = s16[0:8, 0:128]
                        vpu_steps(due(1))
                    emit(u, c * CK + r * 16, s16)
                    st["slab"] += 1
            ot_s[u, pl.ds(hrow, DH), :] = (acc * linv).astype(bf16)
            lbuf[u] = lpart[u]
        return carry + h

    for d in range(DH):
        for j in range(NG):
            kb_s[j, d] = kb_val(0, j, d, 0)
    for c in range(NC):
        make_kh(0, c, 0)
    cnt = lax.fori_loop(0, H, block, jnp.int32(0))

    for u in range(NQ):
        row_sum_inv(u)
    n_bad = jnp.max(bad_s[...])

    @pl.when(n_bad > 0.0)
    def _():
        def one(t, carry):
            h = t // NQ
            u = t % NQ
            hrow = pl.multiple_of(h * DH, DH)
            w = q_weights(u, h)

            def scores(c, m):
                r0 = pl.multiple_of((h // HG) * (S // 2) + c * 64, 64)
                kc = pltpu.roll(k_s[pl.ds(r0, 64), :], shift_of(h), 1)
                s = jnp.dot(pltpu.bitcast(kc, bf16)[:, 0:DH], w, preferred_element_type=f32)
                sbuf[c] = s
                return jnp.maximum(m, jnp.max(s, axis=0, keepdims=True))

            m = lax.fori_loop(0, NC, scores, jnp.full((1, TQ), -jnp.inf, f32))

            def probs(c, l):
                p = jnp.exp2(sbuf[c] - m)
                pbuf[pl.ds(pl.multiple_of(u * (S // 2) + c * 64, 64), 64), :] = _pack(p)
                return l + jnp.sum(p.reshape(CK // 8, 8, TQ), axis=0)

            l = lax.fori_loop(0, NC, probs, jnp.zeros((8, TQ), f32))
            lbuf[u] = l
            acc = pv_chunk(u, h, 0)
            for c in range(1, NC):
                acc = pv_chunk(u, h, c) + acc
            linv = 1.0 / jnp.sum(l, axis=0, keepdims=True)
            ot_s[u, pl.ds(hrow, DH), :] = (acc * linv).astype(bf16)
            return carry

        lax.fori_loop(0, H * NQ, one, 0)

    for cp in late_copies:
        cp.wait()
    NB = TQ // 128
    wo_v = hn_s.at[NQ + lax.shift_right_logical(cnt, 20)]
    pending = []

    def finish(now):
        while pending and pending[0][0] <= now:
            _, t, rb, y = pending.pop(0)
            rows = slice(rb * 128, (rb + 1) * 128)
            h = x_s[pl.ds(t * TQ + rb * 128, 128), :].astype(f32) + y
            h_s[t, rows, :] = h
            hn_s[t, rows, :] = _layernorm(h).astype(bf16)

    pv_state = dict(n=0, acc=None)

    def last_pv(upto):
        while pv_state["n"] < min(upto, NQ * NC):
            u, c = divmod(pv_state["n"], NC)
            pv_state["n"] += 1
            pv = pv_chunk(u, H - 1, c)
            pv_state["acc"] = pv if c == 0 else pv + pv_state["acc"]
            if c == NC - 1:
                linv = 1.0 / jnp.sum(lbuf[u], axis=0, keepdims=True)
                ot_s[u, pl.ds((H - 1) * DH, DH), :] = (pv_state["acc"] * linv).astype(bf16)

    last_pv(NC + PVLEAD)
    for u in range(NQ):
        o_nat = ot_s[u].T
        cols = []
        for c in range(NC):
            n = u * NC + c
            finish(n)
            rb, nt = divmod(c, NB)
            cols.append(jnp.dot(o_nat[rb * 128:(rb + 1) * 128], wo_v[:, nt * 128:(nt + 1) * 128],
                                preferred_element_type=f32))
            last_pv(NC + PVLEAD + n + 1)
            if len(cols) == NB:
                pending.append((n + LNLAG, u, rb, jnp.concatenate(cols, axis=1)))
                cols = []
    finish(10 ** 9)

    def ffn(i, carry):
        rows = pl.ds(aligned(i * TQ, TQ), TQ)
        hn = hn_s[i]
        gate_t = lax.dot_general(wg_s[...], hn, NT, preferred_element_type=f32)
        up_t = lax.dot_general(wu_s[...], hn, NT, preferred_element_type=f32)
        act = (_gelu_tanh(gate_t) * up_t).astype(bf16).T
        for j in range(NO):
            cols = slice(j * (D // NO), (j + 1) * (D // NO))
            y = h_s[i, :, cols] + jnp.dot(act, wd_s[:, cols], preferred_element_type=f32)
            out_s[rows, cols] = y.astype(bf16)
            out_copy(i, j).start()
        return carry

    lax.fori_loop(0, NQ, ffn, 0)
    for i in range(NQ):
        for j in range(NO):
            out_copy(i, j).wait()


@jax.jit
def pallas_sequential_preLN__softmax_full_mha__geglu_ffn__prompt_kernel(
    A_x: jax.Array,
    A_wqkv: jax.Array,
    A_wo: jax.Array,
    B_x: jax.Array,
    B_w_gate: jax.Array,
    B_w_up: jax.Array,
    B_w_down: jax.Array,
):
    del B_x
    hbm_spec = pl.BlockSpec(memory_space=pltpu.HBM)
    out = pl.pallas_call(
        _kernel,
        out_shape=jax.ShapeDtypeStruct((S, D), bf16),
        in_specs=[hbm_spec] * 6,
        out_specs=hbm_spec,
        scratch_shapes=[
            pltpu.VMEM((S, D), bf16),
            pltpu.VMEM((3, D, D), bf16),
            pltpu.VMEM((F, D), bf16),
            pltpu.VMEM((F, D), bf16),
            pltpu.VMEM((F, D), bf16),
            pltpu.VMEM((2 * D, D), bf16),
            pltpu.VMEM(((D // 128) * (S // 2) + 32, 128), u32),
            pltpu.VMEM((S // 2, 128), u32),
            pltpu.VMEM((NQ * D // 2, TQ), u32),
            pltpu.VMEM((NQ, H, DH, 8, TQ), f32),
            pltpu.VMEM((D // 2, S), u32),
            pltpu.VMEM((KB_SRC + 4 * NKF, DH, 16, 128), f32),
            pltpu.VMEM((NQ * S // 2, TQ), u32),
            pltpu.VMEM((NQ, 8, TQ), f32),
            pltpu.VMEM((NQ, 8, TQ), f32),
            pltpu.VMEM((NC, CK, TQ), f32),
            pltpu.VMEM((NQ, D, TQ), bf16),
            pltpu.VMEM((NQ, TQ, D), f32),
            pltpu.VMEM((NQ + 1, TQ, D), bf16),
            pltpu.VMEM((S, D), bf16),
            pltpu.SemaphoreType.DMA((NQ,)),
            pltpu.SemaphoreType.DMA((7,)),
            pltpu.SemaphoreType.DMA((NQ * NO,)),
        ],
        compiler_params=pltpu.CompilerParams(vmem_limit_bytes=110 * 1024 * 1024),
        name="fused_block",
    )(A_x.reshape(S, D), A_wqkv, A_wo, B_w_gate.T, B_w_up.T, B_w_down)
    return out.reshape(1, S, D)
```

```python
import math

import jax
import jax.numpy as jnp
from jax import lax
import jax.experimental.pallas as pl
import jax.experimental.pallas.tpu as pltpu

S, D, H, DH, F = 2048, 512, 32, 16, 1376
TQ = 512
NQ = S // TQ
CK = 128
NC = S // CK
HG = 128 // DH
NO = 2
EPS = 1e-5
QSCALE = (DH ** -0.5) * math.log2(math.e)
L_LO, L_HI = 2.0 ** -50, 2.0 ** 50

NG = 18
LEAD = 10
DELAY = 18
LNLAG = 5
PVLEAD = 6
CNT = [0] * NC
GROW = []
for _j in range(NG):
    _c = max(0, (_j * NC) // NG - 1)
    CNT[_c] += 1
    GROW.append(_c * CK + CK - 16 * CNT[_c])
NSTEP = NG * DH
NSLAB = NC * 8 - NG
NKF = (NG + DH - 1) // DH
KB_TICK = 2 * NG
KB_SRC = 2 * NG + 1

f32, bf16, u32 = jnp.float32, jnp.bfloat16, jnp.uint32
NT = (((1,), (1,)), ((), ()))


def _layernorm(x):
    m = jnp.mean(x, axis=-1, keepdims=True)
    xc = x - m
    v = jnp.mean(xc * xc, axis=-1, keepdims=True)
    return xc * lax.rsqrt(v + EPS)


def _gelu_tanh(x):
    c = math.sqrt(2.0 / math.pi)
    return 0.5 * x * (1.0 + jnp.tanh(c * (x + 0.044715 * (x * x * x))))


def _pack(x):
    return pltpu.bitcast(x.astype(bf16), u32)


def _aligned(v, n):
    return v if isinstance(v, int) else pl.multiple_of(v, n)


def _kernel(x_hbm, wqkv_hbm, wo_hbm, wg_hbm, wu_hbm, wd_hbm, out_hbm,
            x_s, wqkv_s, wg_s, wu_s, wd_s, wqvt_s, k_s, kh_s, qt_s, qf_s, vt_s,
            kb_s, pbuf, lbuf, bad_s, sbuf, ot_s, h_s, hn_s, out_s, sem_x, sem_w, sem_o):
    def x_copy(i):
        return pltpu.make_async_copy(
            x_hbm.at[pl.ds(i * TQ, TQ), :], x_s.at[pl.ds(i * TQ, TQ), :], sem_x.at[i])

    def wqkv_copy(j):
        return pltpu.make_async_copy(
            wqkv_hbm.at[:, pl.ds(j * D, D)], wqkv_s.at[j], sem_w.at[j])

    def out_copy(i, j):
        rows, cols = pl.ds(i * TQ, TQ), pl.ds(j * (D // NO), D // NO)
        return pltpu.make_async_copy(
            out_s.at[rows, cols], out_hbm.at[rows, cols], sem_o.at[i * NO + j])

    late_copies = [
        pltpu.make_async_copy(src, dst, sem_w.at[3 + j])
        for j, (src, dst) in enumerate(
            [(wo_hbm, hn_s.at[NQ]), (wg_hbm, wg_s), (wu_hbm, wu_s), (wd_hbm, wd_s)])
    ]
    x_copy(0).start()
    wqkv_copy(1).start()
    for i in range(1, NQ):
        x_copy(i).start()
    wqkv_copy(0).start()
    wqkv_copy(2).start()

    def ln1(i):
        return _layernorm(x_s[pl.ds(i * TQ, TQ), :].astype(f32)).astype(bf16)

    def proj_k(row0, xn):
        n = xn.shape[0]
        kk = jnp.dot(xn, wqkv_s[1], preferred_element_type=f32)
        for g in range(D // 128):
            k_s[pl.ds(g * (S // 2) + row0 // 2, n // 2), :] = _pack(kk[:, g * 128:(g + 1) * 128])
        for j in range(NG):
            r0 = GROW[j] - row0
            if 0 <= r0 < n:
                for g in range(D // 128):
                    kb_s[KB_SRC + g * NKF + j // DH, j % DH] = kk[r0:r0 + 16, g * 128:(g + 1) * 128]

    def proj_qv(i, xn):
        qv = lax.dot_general(wqvt_s[...], xn, NT, preferred_element_type=f32)
        pbuf[pl.ds(i * (S // 2), S // 2), :] = pltpu.bitcast(qv, u32)
        for h in range(H):
            q = qv[2 * DH * h:2 * DH * h + DH] * QSCALE
            qt_s[pl.ds(i * (D // 2) + h * 8, 8), :] = _pack(q)
            for d in range(DH):
                qf_s[i, h, d] = jnp.broadcast_to(q[d:d + 1], (8, TQ))
            vt_s[pl.ds(h * 8, 8), pl.ds(i * TQ, TQ)] = _pack(qv[2 * DH * h + DH:2 * DH * (h + 1)])

    HT = TQ // 2
    x_copy(0).wait()
    xn0 = ln1(0)
    wqkv_copy(1).wait()
    proj_k(0, xn0[:HT])
    x_copy(1).wait()
    proj_k(HT, xn0[HT:])
    xn1 = ln1(1)
    proj_k(TQ, xn1[:HT])
    x_copy(2).wait()
    proj_k(TQ + HT, xn1[HT:])
    xn2 = ln1(2)
    proj_k(2 * TQ, xn2[:HT])
    x_copy(3).wait()
    wqkv_copy(0).wait()
    wqkv_copy(2).wait()
    for cp in late_copies:
        cp.start()
    proj_k(2 * TQ + HT, xn2[HT:])
    xn3 = ln1(3)
    proj_k(3 * TQ, xn3)
    wq_t, wv_t = wqkv_s[0].T, wqkv_s[2].T
    for h in range(H):
        wqvt_s[2 * DH * h:2 * DH * h + DH, :] = wq_t[h * DH:(h + 1) * DH]
        wqvt_s[2 * DH * h + DH:2 * DH * (h + 1), :] = wv_t[h * DH:(h + 1) * DH]
    for i, xn in enumerate((xn0, xn1, xn2, xn3)):
        proj_qv(i, xn)
    lbuf[...] = jnp.ones(lbuf.shape, f32)
    bad_s[...] = jnp.zeros(bad_s.shape, f32)

    def q_weights(u, h):
        return pltpu.bitcast(qt_s[pl.ds(_aligned(u * (D // 2) + h * 8, 8), 8), :], bf16)

    def shift_of(h):
        return (128 - (h % HG) * DH) % 128

    def kb_val(h, j, d, z):
        kk = kb_s[KB_SRC + (h // HG) * NKF + j // DH + z, j % DH]
        idx = jnp.full((16, 128), (h % HG) * DH + d, jnp.int32)
        return jnp.take_along_axis(kk, idx, axis=1, mode="promise_in_bounds")

    def make_kh(h, c, z):
        n = (CK - 16 * CNT[c]) // 2
        kh_s[pl.ds(c * 64, n), :] = pltpu.roll(
            k_s[pl.ds(_aligned((h // HG + z) * (S // 2), S // 2) + c * 64, n), :], shift_of(h), 1)

    def row_sum_inv(u):
        l = jnp.sum(lbuf[u], axis=0, keepdims=True)
        ok = jnp.logical_and(l >= L_LO, l <= L_HI)
        bad_s[u] = jnp.maximum(bad_s[u], jnp.where(ok, 0.0, 1.0))
        return 1.0 / l

    def pv_chunk(u, h, c):
        p = pltpu.bitcast(pbuf[pl.ds(_aligned(u * (S // 2), 64) + c * 64, 64), :], bf16)
        v = pltpu.bitcast(vt_s[pl.ds(_aligned(h * 8, 8), 8), pl.ds(c * CK, CK)], bf16)
        return jnp.dot(v, p, preferred_element_type=f32)

    def block(h, carry):
        del carry
        h_prep = jnp.minimum(h + 1, H - 1)
        h_prev = jnp.maximum(h - 1, 0)
        hrow = pl.multiple_of(h_prev * DH, DH)
        slot = h % 2
        z = lax.shift_right_logical(h, 20)
        lpart = [None] * NQ
        consumed = set()
        st = dict(acc=None, step=0, slab=0, prod=0)
        queue = []

        def emit(u, row0, s16):
            p = jnp.exp2(s16)
            pair = p[0:8] + p[8:16]
            lpart[u] = pair if lpart[u] is None else lpart[u] + pair
            pbuf[pl.ds(u * (S // 2) + row0 // 2, 8), :] = _pack(p)

        def flush(step):
            while queue and queue[0][0] <= step:
                _, j, d, val = queue.pop(0)
                kb_s[(1 - slot) * NG + j, d] = val

        def vpu_steps(target):
            while st["step"] < target:
                u, n = divmod(st["step"], NSTEP)
                j, d0 = divmod(n, DH)
                cnt = min(target - st["step"], DH - d0)
                st["step"] += cnt
                kb = kb_s[slot * NG + j + z, d0:d0 + cnt]
                kb = jnp.concatenate([kb] * 4, axis=2).reshape(cnt, 2, 8, TQ)
                t = kb * qf_s[u, h, d0:d0 + cnt][:, None]
                for i in range(cnt):
                    st["acc"] = t[i] if d0 + i == 0 else st["acc"] + t[i]
                if d0 + cnt == DH:
                    assert (u, GROW[j] // CK) in consumed
                    emit(u, GROW[j], st["acc"].reshape(16, TQ))
                while st["prod"] * NQ < st["step"]:
                    dd, jj = divmod(st["prod"], NG)
                    queue.append((st["prod"] * NQ + DELAY, jj, dd, kb_val(h_prep, jj, dd, z)))
                    st["prod"] += 1
            if st["step"] == NQ * NSTEP:
                flush(10 ** 9)

        def due(half):
            num = (st["slab"] * 2 + half + LEAD) * NSTEP
            return min(NQ * NSTEP, -(-num // (2 * NSLAB)))

        for u in range(NQ):
            linv = row_sum_inv(u)
            w = q_weights(u, h)
            for c in range(NC):
                nr = CK - 16 * CNT[c]
                kc = pltpu.bitcast(kh_s[pl.ds(c * 64, nr // 2), :], bf16)
                s = jnp.dot(kc[:, 0:DH], w, preferred_element_type=f32)
                if u == NQ - 1:
                    make_kh(h_prep, c, z)
                pv = pv_chunk(u, h_prev, c)
                consumed.add((u, c))
                acc = pv if c == 0 else pv + acc
                if u == 0 and c == 0:
                    vpu_steps(due(0))
                for r in range(nr // 16):
                    s16 = s[r * 16:(r + 1) * 16, :]
                    if r == 0 and (NQ - 2, NC - 2) <= (u, c) < (NQ - 1, NC - 2):
                        k_s[pl.ds((D // 128) * (S // 2), 8), :] = pltpu.bitcast(s16[0:8, 0:128], u32)
                    if st["step"] < due(1):
                        flush(st["step"])
                        kb_s[KB_TICK, 0, 0:8, :] = s16[0:8, 0:128]
                        vpu_steps(due(1))
                    emit(u, c * CK + r * 16, s16)
                    st["slab"] += 1
            assert st["step"] >= (u + 1) * NSTEP
            ot_s[u, pl.ds(hrow, DH), :] = (acc * linv).astype(bf16)
            lbuf[u] = lpart[u]
        return z

    for d in range(DH):
        for j in range(NG):
            kb_s[j, d] = kb_val(0, j, d, 0)
    for c in range(NC):
        make_kh(0, c, 0)
    z_end = lax.fori_loop(0, H, block, jnp.int32(0))

    for u in range(NQ):
        row_sum_inv(u)
    n_bad = jnp.max(bad_s[...])

    @pl.when(n_bad > 0.0)
    def _():
        def one(t, carry):
            h = t // NQ
            u = t % NQ
            w = q_weights(u, h)

            def scores(c, m):
                r0 = pl.multiple_of((h // HG) * (S // 2) + c * 64, 64)
                kc = pltpu.roll(k_s[pl.ds(r0, 64), :], shift_of(h), 1)
                s = jnp.dot(pltpu.bitcast(kc, bf16)[:, 0:DH], w, preferred_element_type=f32)
                sbuf[c] = s
                return jnp.maximum(m, jnp.max(s, axis=0, keepdims=True))

            m = lax.fori_loop(0, NC, scores, jnp.full((1, TQ), -jnp.inf, f32))

            def probs(c, l):
                p = jnp.exp2(sbuf[c] - m)
                pbuf[pl.ds(pl.multiple_of(u * (S // 2) + c * 64, 64), 64), :] = _pack(p)
                return l + jnp.sum(p.reshape(CK // 8, 8, TQ), axis=0)

            l = lax.fori_loop(0, NC, probs, jnp.zeros((8, TQ), f32))
            lbuf[u] = l
            acc = pv_chunk(u, h, 0)
            for c in range(1, NC):
                acc = pv_chunk(u, h, c) + acc
            linv = 1.0 / jnp.sum(l, axis=0, keepdims=True)
            ot_s[u, pl.ds(pl.multiple_of(h * DH, DH), DH), :] = (acc * linv).astype(bf16)
            return carry

        lax.fori_loop(0, H * NQ, one, 0)

    for cp in late_copies:
        cp.wait()
    NB = TQ // 128
    wo_v = hn_s.at[NQ + z_end]
    pending = []
    last = dict(n=0, acc=None)

    def finish(now):
        while pending and pending[0][0] <= now:
            _, t, rb, y = pending.pop(0)
            rows = slice(rb * 128, (rb + 1) * 128)
            h = x_s[pl.ds(t * TQ + rb * 128, 128), :].astype(f32) + y
            h_s[t, rows, :] = h
            hn_s[t, rows, :] = _layernorm(h).astype(bf16)

    def last_pv(upto):
        while last["n"] < min(upto, NQ * NC):
            u, c = divmod(last["n"], NC)
            last["n"] += 1
            pv = pv_chunk(u, H - 1, c)
            last["acc"] = pv if c == 0 else pv + last["acc"]
            if c == NC - 1:
                linv = 1.0 / jnp.sum(lbuf[u], axis=0, keepdims=True)
                ot_s[u, pl.ds((H - 1) * DH, DH), :] = (last["acc"] * linv).astype(bf16)

    last_pv(NC + PVLEAD)
    for u in range(NQ):
        o_nat = ot_s[u].T
        cols = []
        for c in range(NC):
            n = u * NC + c
            finish(n)
            rb, nt = divmod(c, NB)
            cols.append(jnp.dot(o_nat[rb * 128:(rb + 1) * 128], wo_v[:, nt * 128:(nt + 1) * 128],
                                preferred_element_type=f32))
            last_pv(NC + PVLEAD + n + 1)
            if len(cols) == NB:
                pending.append((n + LNLAG, u, rb, jnp.concatenate(cols, axis=1)))
                cols = []
    finish(10 ** 9)

    def ffn(i, carry):
        rows = pl.ds(pl.multiple_of(i * TQ, TQ), TQ)
        hn = hn_s[i]
        gate_t = lax.dot_general(wg_s[...], hn, NT, preferred_element_type=f32)
        up_t = lax.dot_general(wu_s[...], hn, NT, preferred_element_type=f32)
        act = (_gelu_tanh(gate_t) * up_t).astype(bf16).T
        for j in range(NO):
            cols = slice(j * (D // NO), (j + 1) * (D // NO))
            y = h_s[i, :, cols] + jnp.dot(act, wd_s[:, cols], preferred_element_type=f32)
            out_s[rows, cols] = y.astype(bf16)
            out_copy(i, j).start()
        return carry

    lax.fori_loop(0, NQ, ffn, 0)
    for i in range(NQ):
        for j in range(NO):
            out_copy(i, j).wait()


@jax.jit
def pallas_sequential_preLN__softmax_full_mha__geglu_ffn__prompt_kernel(
    A_x: jax.Array,
    A_wqkv: jax.Array,
    A_wo: jax.Array,
    B_x: jax.Array,
    B_w_gate: jax.Array,
    B_w_up: jax.Array,
    B_w_down: jax.Array,
):
    del B_x
    hbm_spec = pl.BlockSpec(memory_space=pltpu.HBM)
    out = pl.pallas_call(
        _kernel,
        out_shape=jax.ShapeDtypeStruct((S, D), bf16),
        in_specs=[hbm_spec] * 6,
        out_specs=hbm_spec,
        scratch_shapes=[
            pltpu.VMEM((S, D), bf16),
            pltpu.VMEM((3, D, D), bf16),
            pltpu.VMEM((F, D), bf16),
            pltpu.VMEM((F, D), bf16),
            pltpu.VMEM((F, D), bf16),
            pltpu.VMEM((2 * D, D), bf16),
            pltpu.VMEM(((D // 128) * (S // 2) + 32, 128), u32),
            pltpu.VMEM((S // 2, 128), u32),
            pltpu.VMEM((NQ * D // 2, TQ), u32),
            pltpu.VMEM((NQ, H, DH, 8, TQ), f32),
            pltpu.VMEM((D // 2, S), u32),
            pltpu.VMEM((KB_SRC + 4 * NKF, DH, 16, 128), f32),
            pltpu.VMEM((NQ * S // 2, TQ), u32),
            pltpu.VMEM((NQ, 8, TQ), f32),
            pltpu.VMEM((NQ, 8, TQ), f32),
            pltpu.VMEM((NC, CK, TQ), f32),
            pltpu.VMEM((NQ, D, TQ), bf16),
            pltpu.VMEM((NQ, TQ, D), f32),
            pltpu.VMEM((NQ + 1, TQ, D), bf16),
            pltpu.VMEM((S, D), bf16),
            pltpu.SemaphoreType.DMA((NQ,)),
            pltpu.SemaphoreType.DMA((7,)),
            pltpu.SemaphoreType.DMA((NQ * NO,)),
        ],
        compiler_params=pltpu.CompilerParams(vmem_limit_bytes=110 * 1024 * 1024),
        name="fused_block",
    )(A_x.reshape(S, D), A_wqkv, A_wo, B_w_gate.T, B_w_up.T, B_w_down)
    return out.reshape(1, S, D)
```
